```python
import os as _os
_os.environ.setdefault('JAX_PLATFORMS', 'cpu')
import jax
import jax.numpy as jnp

def _softmax(x, axis=-1):
    return jax.nn.softmax(x, axis=axis)

def _gelu(x):
    return jax.nn.gelu(x, approximate=True)

def _silu(x):
    return jax.nn.silu(x)

def _sigmoid(x):
    return jax.nn.sigmoid(x)

def _layernorm(x, axis=-1, eps=1e-05):
    m = jnp.mean(x, axis=axis, keepdims=True)
    v = jnp.var(x, axis=axis, keepdims=True)
    return (x - m) / jnp.sqrt(v + eps)

def _scatter_add(tgt, idx, src, axis=0):
    return tgt.at[idx].add(src)

def _segment_sum(src, seg, n):
    return jax.ops.segment_sum(src, seg, n)

class _Rng:

    def __init__(self, key):
        self._k = key

    def _next(self):
        self._k, sub = jax.random.split(self._k)
        return sub

    def normal(self, shape):
        return jax.random.normal(self._next(), shape, dtype=jnp.bfloat16)

    def randint(self, lo, hi, shape):
        return jax.random.randint(self._next(), shape, lo, hi, dtype=jnp.int32)

    def uniform(self, shape, lo=0.0, hi=1.0):
        return jax.random.uniform(self._next(), shape, jnp.bfloat16, lo, hi)

    def permutation(self, n):
        return jax.random.permutation(self._next(), n)
kernel_name = 'adaLN_cond__linear_kernel_hedgehog__geglu_ffn__prompt'

def setup_inputs():
    _rng = _Rng(jax.random.key(int.from_bytes(__import__("os").urandom(4), "little")))
    _w = lambda a: (lambda t: t.astype(jnp.bfloat16) if jnp.issubdtype(t.dtype, jnp.floating) else t)(jnp.asarray(a))

    def _A_setup():
        B, S, D, H = (1, 2048, 512, 32)
        Dh = D // H
        return {'x': _w((lambda *s: _rng.normal(s) * 0.05)(B, S, D)), 'wqkv': _w((lambda *s: _rng.normal(s) * 0.4)(D, 3 * D)), 'w_phi': _w((lambda *s: _rng.normal(s) * 0.4)(H, Dh, Dh) * Dh ** (-0.5)), 'wo': _w((lambda *s: _rng.normal(s) * 0.05)(D, D))}
    _A_in = _A_setup()

    def _B_setup():
        B, S, D, F = (1, 2048, 512, 1792)
        return {'x': _w((lambda *s: _rng.normal(s) * 0.05)(B, S, D)), 'w_gate': _w((lambda *s: _rng.normal(s) * 0.05)(D, F)), 'w_up': _w((lambda *s: _rng.normal(s) * 0.05)(D, F)), 'w_down': _w((lambda *s: _rng.normal(s) * 0.05)(F, D))}
    _B_in = _B_setup()
    return {'A_x': _A_in['x'], 'A_wqkv': _A_in['wqkv'], 'A_w_phi': _A_in['w_phi'], 'A_wo': _A_in['wo'], 'B_x': _B_in['x'], 'B_w_gate': _B_in['w_gate'], 'B_w_up': _B_in['w_up'], 'B_w_down': _B_in['w_down'], 'c': _w((lambda *s: _rng.normal(s) * 0.05)(1, 512) * 8.0), 'w_mod': _w((lambda *s: _rng.normal(s) * 0.05)(512, 6 * 512) * 512 ** (-0.5) * 8.0)}

def reference(A_x, A_wqkv, A_w_phi, A_wo, B_x, B_w_gate, B_w_up, B_w_down, c, w_mod):

    def _A_ref(x, wqkv, w_phi, wo):
        B, S, D = x.shape
        H = 32
        Dh = D // H
        qkv = (lambda x, *d: x.transpose(*d))((x @ wqkv).reshape(B, S, 3, H, Dh), 2, 0, 3, 1, 4)
        q, k, v = (qkv[0], qkv[1], qkv[2])
        pq = jnp.einsum('bhsd,hdf->bhsf', q, w_phi)
        pk = jnp.einsum('bhsd,hdf->bhsf', k, w_phi)
        phi_q = jnp.concatenate([_softmax(pq, axis=-1), _softmax(-pq, axis=-1)], axis=-1)
        phi_k = jnp.concatenate([_softmax(pk, axis=-1), _softmax(-pk, axis=-1)], axis=-1)
        kv = jnp.einsum('bhsf,bhsd->bhfd', phi_k, v)
        z = jnp.einsum('bhsf->bhf', phi_k)
        num = jnp.einsum('bhqf,bhfd->bhqd', phi_q, kv)
        den = jnp.einsum('bhqf,bhf->bhq', phi_q, z)[..., None] + 1e-06
        o = num / den
        return (lambda x, *d: x.transpose(*d))(o, 0, 2, 1, 3).reshape(B, S, D) @ wo

    def _B_ref(x, w_gate, w_up, w_down):
        return _gelu(x @ w_gate) * (x @ w_up) @ w_down
    x = A_x
    mod = (_silu(c) @ w_mod).reshape(c.shape[0], 6, 1, -1)
    sa, ca, ga, sb, cb, gb = (mod[:, 0].copy(), mod[:, 1].copy(), mod[:, 2].copy(), mod[:, 3].copy(), mod[:, 4].copy(), mod[:, 5].copy())
    h = _layernorm(x, axis=-1) * (1 + ca) + sa
    x = x + ga * _A_ref(h, A_wqkv, A_w_phi, A_wo)
    h = _layernorm(x, axis=-1) * (1 + cb) + sb
    x = x + gb * _B_ref(h, B_w_gate, B_w_up, B_w_down)
    return x
```

```python
import jax
import jax.numpy as jnp
import jax.experimental.pallas as pl
import jax.experimental.pallas.tpu as pltpu

S, D, F, T = 2048, 512, 1792, 256
FC = 256
f32, bf = jnp.float32, jnp.bfloat16
NN = (((1,), (0,)), ((), ()))
NT = (((1,), (1,)), ((), ()))
TN = (((0,), (0,)), ((), ()))


def dot(a, b, dn=NN):
    return jax.lax.dot_general(a, b, dn, preferred_element_type=f32)


def ln(x):
    d = x - jnp.mean(x, -1, keepdims=True)
    return d * jax.lax.rsqrt(jnp.mean(d * d, -1, keepdims=True) + 1e-5)


def iot(sh, d):
    return jax.lax.broadcasted_iota(jnp.int32, sh, d)


def comb(op, y):
    return op(y, pltpu.roll(y, 4, 0))


def feats(p):
    p = p.reshape(8, 8, p.shape[-1])
    a = jnp.exp(p - comb(jnp.maximum, jnp.max(p, 0))[None])
    b = jnp.exp(comb(jnp.minimum, jnp.min(p, 0))[None] - p)
    return (a * (1.0 / comb(jnp.add, jnp.sum(a, 0)))[None],
            b * (1.0 / comb(jnp.add, jnp.sum(b, 0)))[None])


def body(x_h, wqkv_h, phi_h, wo_h, wg_h, wu_h, wd_h, c_h, wm_h, o_h,
         x, wqkv, phi, wo, wg, wu, wd, c, wm, ob, hb, x1s, h2s, mod, wt, wop, kv, kvb, z,
         sem, osem):
    N = S // T
    cp = lambda s, d, n: pltpu.make_async_copy(s, d, sem.at[n])
    col = lambda r, a, n: r.at[:, pl.ds(a, n)]
    c_c, c_phi = cp(c_h, c, 0), cp(phi_h, phi, 1)
    c_m0 = cp(col(wm_h, 0, 2 * D), col(wm, 0, 2 * D), 2)
    c_m1 = cp(col(wm_h, 2 * D, 4 * D), col(wm, 2 * D, 4 * D), 3)
    c_w = [cp(col(wqkv_h, s * D, D), col(wqkv, s * D, D), 4 + s) for s in range(3)]
    c_o, c_g, c_u, c_d = cp(wo_h, wo, 7), cp(wg_h, wg, 8), cp(wu_h, wu, 9), cp(wd_h, wd, 10)
    c_x = [cp(x_h.at[pl.ds(a, n)], x.at[pl.ds(a, n)], 11 + i) for i, (a, n) in enumerate(((0, T), (T, 2 * T), (3 * T, S - 3 * T)))]
    rows = lambda i: pl.ds(i * T if isinstance(i, int) else pl.multiple_of(i * T, T), T)

    for d in (c_c, c_phi, c_x[0], c_m0, c_w[1]):
        d.start()
    c_c.wait()
    cc = jnp.broadcast_to(c[...].astype(f32), (8, D))
    sc = (cc * jax.nn.sigmoid(cc)).astype(bf)
    c_phi.wait()
    r_, c_ = iot((128, 128), 0), iot((128, 128), 1)
    mk = (r_ // 64 * 4 + r_ % 4) == c_ // 16
    et = (iot((128, 16), 0) % 64 // 4 == iot((128, 16), 1)).astype(bf)
    mphi = [jnp.where(mk, dot(et, phi[j * 128:(j + 1) * 128, :], NT), 0.0).astype(bf) for j in range(4)]
    perm = (mk & (r_ % 64 // 4 == c_ % 16)).astype(bf)
    kv[...] = jnp.zeros_like(kv)
    z[...] = jnp.zeros_like(z)

    def fold(s):
        for j in range(4):
            r = s * D + j * 128
            m = perm if s == 2 else mphi[j]
            wt[r:r + 128, :] = dot(m, wqkv[:, r:r + 128], NT).astype(bf)

    def ln1(i):
        xf = x[rows(i), :].astype(f32)
        hb[rows(i), :] = (ln(xf) * (1 + mod[0:1, D:2 * D]) + mod[0:1, :D]).astype(bf)

    c_m0.wait()
    c_w[2].start()
    c_x[1].start()
    c_x[2].start()
    mod[:, :2 * D] = dot(sc, wm[:, :2 * D])
    c_x[0].wait()
    ln1(0)
    c_w[1].wait()
    fold(1)
    proj = lambda s, i: dot(wt[s * D:(s + 1) * D, :], hb[rows(i), :], NT)
    pk = proj(1, 0)
    for i in range(N):
        abs_ = []
        for g in range(8):
            a, b = feats(pk[g * 64:(g + 1) * 64])
            z[g, 0] += sum(a[:, :, t:t + 128] for t in range(0, T, 128))
            z[g, 1] += sum(b[:, :, t:t + 128] for t in range(0, T, 128))
            abs_.append(jnp.concatenate([a.reshape(64, T), b.reshape(64, T)], 0).astype(bf))
        if i == 0:
            c_w[2].wait()
            c_x[1].wait()
            fold(2)
            ln1(1)
        if i == 1:
            c_x[2].wait()
            for d in (c_w[0], c_m1, c_o, c_g, c_u, c_d):
                d.start()
        if i == N - 2:
            c_w[0].wait()
            c_m1.wait()
            c_o.wait()
            fold(0)
            mod[:, 2 * D:] = dot(sc, wm[:, 2 * D:])
            for j in range(4):
                wop[j * 128:(j + 1) * 128, :] = dot(perm, wo[j * 128:(j + 1) * 128, :]).astype(bf)
        if i == N - 1:
            pq0 = proj(0, 0)
        if i + 2 < N:
            ln1(i + 2)
        vt = proj(2, i).astype(bf)
        if i + 1 < N:
            pk = proj(1, i + 1)
        for g in range(8):
            kv[g] += dot(vt[g * 64:(g + 1) * 64], abs_[g], NT)

    km = iot((64, 128), 0) % 4 == iot((64, 128), 1) % 4
    for g in range(8):
        kvb[g] = jnp.where(km, kv[g], 0.0).astype(bf)
        for s in range(2):
            z[g, s] = jnp.broadcast_to(jnp.sum(z[g, s], -1, keepdims=True), (8, 8, 128))

    def attn(i, slot, pq=None):
        if pq is None:
            pq = proj(0, i)
        os = []
        for g in range(8):
            a, b = feats(pq[g * 64:(g + 1) * 64])
            za = jnp.concatenate([z[g, 0]] * (T // 128), -1)
            zb = jnp.concatenate([z[g, 1]] * (T // 128), -1)
            r = 1.0 / (comb(jnp.add, jnp.sum(a * za + b * zb, 0)) + 1e-6)
            ab = jnp.concatenate([a.reshape(64, T), b.reshape(64, T)], 0).astype(bf)
            o = dot(kvb[g], ab).reshape(8, 8, T) * r[None]
            os.append(o.reshape(64, T).astype(bf))
        x1 = x[rows(i), :].astype(f32) + mod[0:1, 2 * D:3 * D] * dot(jnp.concatenate(os, 0), wop[...], TN)
        x1s[slot] = x1
        h2s[slot] = (ln(x1) * (1 + mod[0:1, 4 * D:5 * D]) + mod[0:1, 3 * D:4 * D]).astype(bf)

    def ffn(i, slot):
        h = h2s[slot]
        acts = []
        for k in range(0, F, FC):
            g = dot(h, wg[:, k:k + FC])
            u = dot(h, wu[:, k:k + FC])
            acts.append((jax.nn.gelu(g, approximate=True) * u).astype(bf))
        y = dot(jnp.concatenate(acts, 1), wd[...])
        ob[rows(i), :] = (x1s[slot] + mod[0:1, 5 * D:] * y).astype(ob.dtype)
        pltpu.make_async_copy(ob.at[rows(i)], o_h.at[rows(i)], osem.at[i]).start()

    attn(0, 0, pq0)
    for d in (c_g, c_u, c_d):
        d.wait()

    def step(i, carry):
        attn(i + 1, (i + 1) % 2)
        ffn(i, i % 2)
        return carry

    jax.lax.fori_loop(0, N - 1, step, 0)
    ffn(N - 1, (N - 1) % 2)
    for i in range(N):
        pltpu.make_async_copy(ob.at[rows(i)], o_h.at[rows(i)], osem.at[i]).wait()


@jax.jit
def pallas_adaLN_cond__linear_kernel_hedgehog__geglu_ffn__prompt_kernel(
        A_x, A_wqkv, A_w_phi, A_wo, B_x, B_w_gate, B_w_up, B_w_down, c, w_mod):
    hbm = pl.BlockSpec(memory_space=pltpu.MemorySpace.HBM)
    V = pltpu.VMEM
    ins = (A_x.reshape(S, D), A_wqkv, A_w_phi.reshape(D, 16), A_wo, B_w_gate, B_w_up, B_w_down, c, w_mod)
    return pl.pallas_call(
        body,
        in_specs=[hbm] * 9,
        out_specs=hbm,
        out_shape=jax.ShapeDtypeStruct((S, D), A_x.dtype),
        scratch_shapes=[V(a.shape, a.dtype) for a in ins] + [
            V((S, D), A_x.dtype), V((S, D), bf), V((2, T, D), f32), V((2, T, D), bf),
            V((8, 6 * D), f32), V((3 * D, D), bf), V((D, D), bf),
            V((8, 64, 128), f32), V((8, 64, 128), bf), V((8, 2, 8, 8, 128), f32),
            pltpu.SemaphoreType.DMA((14,)), pltpu.SemaphoreType.DMA((S // T,))],
        compiler_params=pltpu.CompilerParams(vmem_limit_bytes=100 << 20),
    )(*ins).reshape(1, S, D)
```
